```python
import jax
import jax.numpy as jnp

def _softmax(x, axis=-1):
    return jax.nn.softmax(x, axis=axis)
def _gelu(x):
    return jax.nn.gelu(x, approximate=True)
def _silu(x):
    return jax.nn.silu(x)
def _sigmoid(x):
    return jax.nn.sigmoid(x)
def _layernorm(x, axis=-1, eps=1e-5):
    m = jnp.mean(x, axis=axis, keepdims=True)
    v = jnp.var(x, axis=axis, keepdims=True)
    return (x - m) / jnp.sqrt(v + eps)
def _scatter_add(tgt, idx, src, axis=0):
    return tgt.at[idx].add(src)
def _segment_sum(src, seg, n):
    return jax.ops.segment_sum(src, seg, n)
class _Rng:
    def __init__(self, key):
        self._k = key
    def _next(self):
        self._k, sub = jax.random.split(self._k)
        return sub
    def normal(self, shape):
        return jax.random.normal(self._next(), shape, dtype=jnp.bfloat16)
    def randint(self, lo, hi, shape):
        return jax.random.randint(self._next(), shape, lo, hi, dtype=jnp.int32)
    def uniform(self, shape, lo=0.0, hi=1.0):
        return jax.random.uniform(self._next(), shape, jnp.bfloat16, lo, hi)
    def permutation(self, n):
        return jax.random.permutation(self._next(), n)


kernel_name = 'parallel_sum__sliding_block_cached__moe_arch_mod__decode'

def setup_inputs():
    _rng = _Rng(jax.random.key(int.from_bytes(__import__("os").urandom(4), "little")))
    _w = (lambda a: (lambda t: t.astype(jnp.bfloat16) if jnp.issubdtype(t.dtype, jnp.floating) else t)(jnp.asarray(a)))
    def _A_setup():
        B, Sq, D = 1, 1, 512
        Hq, Hkv, Sk, Dh = 32, 8, 65536, 128
        assert Hq % Hkv == 0, (Hq, Hkv)
        return {
            "x": _w((lambda *s: _rng.normal(s) * 0.05)(B, Sq, D)),
            "k_cache": _w((lambda *s: _rng.normal(s) * 0.05)(B, Hkv, Sk, Dh)),
            "v_cache": _w((lambda *s: _rng.normal(s) * 0.05)(B, Hkv, Sk, Dh)),
            "wq": _w((lambda *s: _rng.normal(s) * 0.05)(D, Hq * Dh) * (D ** -0.5)),
            "wo": _w((lambda *s: _rng.normal(s) * 0.05)(Hq * Dh, D) * ((Hq * Dh) ** -0.5)),
        }
    _A_in = _A_setup()

    def _B_setup():
        B, S, D, F, C = 1, 1, 512, 1792, 1
        return {
            "x": _w((lambda *s: _rng.normal(s) * 0.05)(B, S, D)),
            "w_r": _w((lambda *s: _rng.normal(s) * 0.05)(D)),
            "w_gate": _w((lambda *s: _rng.normal(s) * 0.05)(D, F)),
            "w_up": _w((lambda *s: _rng.normal(s) * 0.05)(D, F)),
            "w_down": _w((lambda *s: _rng.normal(s) * 0.05)(F, D)),
        }
    _B_in = _B_setup()

    return {
        "A_x": _A_in["x"],
        "A_k_cache": _A_in["k_cache"],
        "A_v_cache": _A_in["v_cache"],
        "A_wq": _A_in["wq"],
        "A_wo": _A_in["wo"],
        "B_x": _B_in["x"],
        "B_w_r": _B_in["w_r"],
        "B_w_gate": _B_in["w_gate"],
        "B_w_up": _B_in["w_up"],
        "B_w_down": _B_in["w_down"],
    }

def reference(A_x, A_k_cache, A_v_cache, A_wq, A_wo, B_x, B_w_r, B_w_gate, B_w_up, B_w_down):
    def _A_ref(x, k_cache, v_cache, wq, wo):
        B, Sq, D = x.shape
        Hq, Dh = 32, 128
        Hkv, Sk = k_cache.shape[1], k_cache.shape[2]
        W = min(4096, max(256, Sk // 4))
        rep = Hq // Hkv
        q = (lambda x, *d: x.transpose(*d))((x @ wq).reshape(B, Sq, Hq, Dh), 0, 2, 1, 3)
        k = jnp.repeat(k_cache[:, :, Sk - W:, :], rep, axis=1)
        v = jnp.repeat(v_cache[:, :, Sk - W:, :], rep, axis=1)
        scores = jnp.einsum("bhqd,bhkd->bhqk", q, k) * (Dh ** -0.5)
        p = _softmax(scores, axis=-1)
        o = jnp.einsum("bhqk,bhkd->bhqd", p, v)
        return (lambda x, *d: x.transpose(*d))(o, 0, 2, 1, 3).reshape(B, Sq, Hq * Dh) @ wo

    def _B_ref(x, w_r, w_gate, w_up, w_down):
        B, S, D = x.shape
        C = 1
        r = x @ w_r
        idx = jnp.argsort(-r, axis=-1)[:, :C]
        idx_e = jnp.repeat(idx.reshape(B, C, 1), D, axis=2)
        x_sel = jnp.take_along_axis(x, idx_e, axis=1)
        g = _silu(x_sel @ w_gate)
        u = x_sel @ w_up
        y = (g * u) @ w_down
        r_sel = _sigmoid(jnp.take_along_axis(r, idx, axis=1))
        y = y * r_sel.reshape(B, C, 1)
        b_off = (jnp.arange(B) * S).reshape(B, 1)
        flat_idx = (idx + b_off).reshape(B * C)
        zero = (x * 0.0).reshape(B * S, D)
        upd = _scatter_add(zero, flat_idx, y.reshape(B * C, D), axis=0)
        return x + upd.reshape(B, S, D)

    x = A_x
    xn = _layernorm(x, axis=-1)
    return x + _A_ref(xn, A_k_cache, A_v_cache, A_wq, A_wo) + _B_ref(xn, B_w_r, B_w_gate, B_w_up, B_w_down)
```

```python
import jax
import jax.numpy as jnp
from jax import lax
import jax.experimental.pallas as pl
import jax.experimental.pallas.tpu as pltpu

_F32 = jnp.float32
_BF16 = jnp.bfloat16
_NT = (((1,), (1,)), ((), ()))

_D = 512
_F = 1792
_HQ, _HKV, _DH = 32, 8, 128
_REP = _HQ // _HKV
_SK = 65536
_W = min(4096, max(256, _SK // 4))
_GW = _REP * _DH
_WD_CHUNKS = 2


def _kernel(x_hbm, wr_hbm, k_hbm, v_hbm, wq_hbm, wo_hbm, wg_hbm, wu_hbm, wd_hbm, o_ref,
            x_v, wr_v, k_v, v_v, wq_v, wo_v, wg_v, wu_v, wd_v, sems):
    cps = {}

    def fetch(name, src, dst):
        c = pltpu.make_async_copy(src, dst, sems.at[len(cps)])
        cps[name] = c
        c.start()

    fetch("x", x_hbm, x_v)
    fetch("wr", wr_hbm, wr_v)
    for h in range(_HKV):
        cols = pl.ds(h * _GW, _GW)
        fetch(("wq", h), wq_hbm.at[:, cols], wq_v.at[:, cols])
        fetch(("k", h), k_hbm.at[0, h, pl.ds(_SK - _W, _W)], k_v.at[h])
        fetch(("v", h), v_hbm.at[0, h, pl.ds(_SK - _W, _W)], v_v.at[h])
        fetch(("wo", h), wo_hbm.at[cols, :], wo_v.at[cols, :])
    fetch("wg", wg_hbm, wg_v)
    fetch("wu", wu_hbm, wu_v)
    fc = _F // _WD_CHUNKS
    for i in range(_WD_CHUNKS):
        rows = pl.ds(i * fc, fc)
        fetch(("wd", i), wd_hbm.at[rows], wd_v.at[rows])

    cps["x"].wait()
    cps["wr"].wait()
    x = x_v[0].astype(_F32)
    wr = wr_v[...].astype(_F32).reshape(1, _D)
    mean = jnp.mean(x, axis=-1, keepdims=True)
    xc = x - mean
    var = jnp.mean(xc * xc, axis=-1, keepdims=True)
    xn = (xc / jnp.sqrt(var + 1e-5)).astype(_BF16).astype(_F32)
    r = jnp.sum(xn * wr, axis=-1, keepdims=True)
    x8 = jnp.broadcast_to(xn, (8, _D)).astype(_BF16)
    row = lax.broadcasted_iota(jnp.int32, (8, _DH), 0)

    acc = jnp.zeros((8, _D), _F32)
    for h in range(_HKV):
        cps[("wq", h)].wait()
        qf = jnp.dot(x8, wq_v[:, h * _GW:(h + 1) * _GW], preferred_element_type=_F32)
        q = jnp.zeros((8, _DH), _F32)
        for j in range(_REP):
            q = jnp.where(row == j, qf[:, j * _DH:(j + 1) * _DH], q)
        cps[("k", h)].wait()
        s = lax.dot_general(q.astype(_BF16), k_v[h], _NT, preferred_element_type=_F32)
        s = s * (_DH ** -0.5)
        p = jnp.exp(s - jnp.max(s, axis=-1, keepdims=True))
        l = jnp.sum(p, axis=-1, keepdims=True)
        cps[("v", h)].wait()
        o = jnp.dot(p.astype(_BF16), v_v[h], preferred_element_type=_F32) / l
        obd = jnp.concatenate([jnp.where(row == j, o, 0.0) for j in range(_REP)], axis=-1)
        cps[("wo", h)].wait()
        acc = acc + jnp.dot(obd.astype(_BF16), wo_v[h * _GW:(h + 1) * _GW, :],
                            preferred_element_type=_F32)
    attn = jnp.sum(acc, axis=0, keepdims=True)

    cps["wg"].wait()
    g = jnp.dot(x8, wg_v[...], preferred_element_type=_F32)
    g = g * jax.nn.sigmoid(g)
    cps["wu"].wait()
    u = jnp.dot(x8, wu_v[...], preferred_element_type=_F32)
    hid = (g * u).astype(_BF16)
    y = jnp.zeros((8, _D), _F32)
    for i in range(_WD_CHUNKS):
        cps[("wd", i)].wait()
        y = y + jnp.dot(hid[:, i * fc:(i + 1) * fc], wd_v[i * fc:(i + 1) * fc, :],
                        preferred_element_type=_F32)
    upd = xn * 0.0 + y[0:1] * jax.nn.sigmoid(r)
    o_ref[0] = (x + attn + (xn + upd)).astype(o_ref.dtype)


@jax.jit
def pallas_parallel_sum__sliding_block_cached__moe_arch_mod__decode_kernel(
    A_x: jax.Array,
    A_k_cache: jax.Array,
    A_v_cache: jax.Array,
    A_wq: jax.Array,
    A_wo: jax.Array,
    B_x: jax.Array,
    B_w_r: jax.Array,
    B_w_gate: jax.Array,
    B_w_up: jax.Array,
    B_w_down: jax.Array,
):
    del B_x
    hbm = pl.BlockSpec(memory_space=pl.ANY)
    n_sems = 2 + 4 * _HKV + 2 + _WD_CHUNKS
    return pl.pallas_call(
        _kernel,
        out_shape=jax.ShapeDtypeStruct((1, 1, _D), _BF16),
        in_specs=[hbm] * 9,
        out_specs=pl.BlockSpec(memory_space=pltpu.VMEM),
        scratch_shapes=[
            pltpu.VMEM((1, 1, _D), _BF16),
            pltpu.VMEM((_D,), _BF16),
            pltpu.VMEM((_HKV, _W, _DH), _BF16),
            pltpu.VMEM((_HKV, _W, _DH), _BF16),
            pltpu.VMEM((_D, _HQ * _DH), _BF16),
            pltpu.VMEM((_HQ * _DH, _D), _BF16),
            pltpu.VMEM((_D, _F), _BF16),
            pltpu.VMEM((_D, _F), _BF16),
            pltpu.VMEM((_F, _D), _BF16),
            pltpu.SemaphoreType.DMA((n_sems,)),
        ],
        compiler_params=pltpu.CompilerParams(vmem_limit_bytes=64 * 1024 * 1024),
    )(A_x, B_w_r, A_k_cache, A_v_cache, A_wq, A_wo, B_w_gate, B_w_up, B_w_down)
```

```python
import jax
import jax.numpy as jnp
from jax import lax
import jax.experimental.pallas as pl
import jax.experimental.pallas.tpu as pltpu

_F32 = jnp.float32
_BF16 = jnp.bfloat16
_NT = (((1,), (1,)), ((), ()))

_D = 512
_F = 1792
_HQ, _HKV, _DH = 32, 8, 128
_REP = _HQ // _HKV
_SK = 65536
_W = min(4096, max(256, _SK // 4))
_GW = _REP * _DH

_WD_MXU = (1408, 256)
_WD_VPU = (96, 32)
_WD_PIECES = _WD_MXU + _WD_VPU
_WD_OFFS = tuple(sum(_WD_PIECES[:i]) for i in range(len(_WD_PIECES) + 1))
assert _WD_OFFS[-1] == _F and sum(_WD_VPU) == 128
_N_SEMS = 1 + _HKV + 1 + len(_WD_PIECES)


def _body(x_hbm, wr_hbm, k_hbm, v_hbm, wq_hbm, wo_hbm, wg_hbm, wu_hbm, wd_hbm, o_ref,
          x_v, wr_v, k_v, v_v, wq_v, wo_v, wg_v, wu_v, wd_v, y_v, ht_v, sems):

    def head_group(h):
        start = h * _GW if isinstance(h, int) else pl.multiple_of(h * _GW, _GW)
        cols = pl.ds(start, _GW)
        pairs = [(wq_hbm.at[:, cols], wq_v.at[h]),
                 (k_hbm.at[0, h, pl.ds(_SK - _W, _W)], k_v.at[h]),
                 (v_hbm.at[0, h, pl.ds(_SK - _W, _W)], v_v.at[h]),
                 (wo_hbm.at[cols, :], wo_v.at[h])]
        return [pltpu.make_async_copy(s, d, sems.at[1 + h]) for s, d in pairs]

    small = [pltpu.make_async_copy(s, d, sems.at[0]) for s, d in ((x_hbm, x_v), (wr_hbm, wr_v))]
    gate_up = [pltpu.make_async_copy(s, d, sems.at[1 + _HKV])
               for s, d in ((wg_hbm, wg_v), (wu_hbm, wu_v))]
    down = []
    for i, c in enumerate(_WD_PIECES):
        rows = pl.ds(_WD_OFFS[i], c)
        down.append(pltpu.make_async_copy(wd_hbm.at[rows], wd_v.at[rows], sems.at[2 + _HKV + i]))

    for c in small:
        c.start()
    for h in range(_HKV):
        for c in head_group(h):
            c.start()
    for c in gate_up + down:
        c.start()

    for c in small:
        c.wait()
    x = x_v[0].astype(_F32)
    wr = wr_v[...].astype(_F32).reshape(1, _D)
    mean = jnp.mean(x, axis=-1, keepdims=True)
    xc = x - mean
    var = jnp.mean(xc * xc, axis=-1, keepdims=True)
    xn = (xc / jnp.sqrt(var + 1e-5)).astype(_BF16).astype(_F32)
    r = jnp.sum(xn * wr, axis=-1, keepdims=True)
    x8 = jnp.broadcast_to(xn, (8, _D)).astype(_BF16)
    row = lax.broadcasted_iota(jnp.int32, (8, _DH), 0)

    def head(h, acc):
        for c in head_group(h):
            c.wait()
        qf = jnp.dot(x8, wq_v[h], preferred_element_type=_F32)
        q = jnp.zeros((8, _DH), _F32)
        for j in range(_REP):
            q = jnp.where(row == j, qf[:, j * _DH:(j + 1) * _DH], q)
        s = lax.dot_general(q.astype(_BF16), k_v[h], _NT, preferred_element_type=_F32)
        s = s * (_DH ** -0.5)
        p = jnp.exp(s - jnp.max(s, axis=-1, keepdims=True))
        l = jnp.sum(p, axis=-1, keepdims=True)
        o = jnp.dot(p.astype(_BF16), v_v[h], preferred_element_type=_F32) / l
        obd = jnp.concatenate([jnp.where(row == j, o, 0.0) for j in range(_REP)], axis=-1)
        return acc + jnp.dot(obd.astype(_BF16), wo_v[h], preferred_element_type=_F32)

    acc = lax.fori_loop(0, _HKV, head, jnp.zeros((8, _D), _F32))
    attn = jnp.sum(acc, axis=0, keepdims=True)

    base = x + attn + (xn + xn * 0.0)
    sig = jax.nn.sigmoid(r)
    for c in gate_up:
        c.wait()
    g = jnp.dot(x8, wg_v[...], preferred_element_type=_F32)
    g = g * jax.nn.sigmoid(g)
    u = jnp.dot(x8, wu_v[...], preferred_element_type=_F32)
    hid = (g * u).astype(_BF16)
    tail = hid[0:1, _F - 128:_F].astype(_F32) * sig
    ht_v[...] = jnp.broadcast_to(tail, (128, 128)).T

    row8 = lax.broadcasted_iota(jnp.int32, (8, _D), 0)
    for i, c in enumerate(_WD_PIECES):
        lo = _WD_OFFS[i]
        down[i].wait()
        if i < len(_WD_MXU):
            y = jnp.dot(hid[:, lo:lo + c], wd_v[lo:lo + c, :], preferred_element_type=_F32)
            if i > 0:
                y = y + y_v[...]
            if i == len(_WD_MXU) - 1:
                y = jnp.where(row8 == 0, y * sig + base, 0.0)
        else:
            k0 = lo - (_F - 128)
            ht4 = jnp.concatenate([ht_v[k0:k0 + c, :]] * (_D // 128), axis=-1)
            w = wd_v[lo:lo + c, :].astype(_F32)
            y = y_v[...] + (w * ht4).reshape(c // 8, 8, _D).sum(axis=0)
        if i < len(_WD_PIECES) - 1:
            y_v[...] = y
    o_ref[0] = jnp.sum(y, axis=0, keepdims=True).astype(o_ref.dtype)


def _kernel(*refs):
    pl.run_scoped(lambda sems: _body(*refs, sems), pltpu.SemaphoreType.DMA((_N_SEMS,)))


@jax.jit
def pallas_parallel_sum__sliding_block_cached__moe_arch_mod__decode_kernel(
    A_x: jax.Array,
    A_k_cache: jax.Array,
    A_v_cache: jax.Array,
    A_wq: jax.Array,
    A_wo: jax.Array,
    B_x: jax.Array,
    B_w_r: jax.Array,
    B_w_gate: jax.Array,
    B_w_up: jax.Array,
    B_w_down: jax.Array,
):
    del B_x
    hbm = pl.BlockSpec(memory_space=pl.ANY)
    return pl.pallas_call(
        _kernel,
        out_shape=jax.ShapeDtypeStruct((1, 1, _D), _BF16),
        in_specs=[hbm] * 9,
        out_specs=pl.BlockSpec(memory_space=pltpu.VMEM),
        scratch_shapes=[
            pltpu.VMEM((1, 1, _D), _BF16),
            pltpu.VMEM((_D,), _BF16),
            pltpu.VMEM((_HKV, _W, _DH), _BF16),
            pltpu.VMEM((_HKV, _W, _DH), _BF16),
            pltpu.VMEM((_HKV, _D, _GW), _BF16),
            pltpu.VMEM((_HKV, _GW, _D), _BF16),
            pltpu.VMEM((_D, _F), _BF16),
            pltpu.VMEM((_D, _F), _BF16),
            pltpu.VMEM((_F, _D), _BF16),
            pltpu.VMEM((8, _D), _F32),
            pltpu.VMEM((128, 128), _F32),
        ],
        compiler_params=pltpu.CompilerParams(vmem_limit_bytes=64 * 1024 * 1024),
    )(A_x, B_w_r, A_k_cache, A_v_cache, A_wq, A_wo, B_w_gate, B_w_up, B_w_down)
```
